```python
import os as _os
_os.environ.setdefault("JAX_PLATFORMS", "cpu")
import jax
import jax.numpy as jnp

def _softmax(x, axis=-1):
    return jax.nn.softmax(x, axis=axis)
def _gelu(x):
    return jax.nn.gelu(x, approximate=True)
def _silu(x):
    return jax.nn.silu(x)
def _sigmoid(x):
    return jax.nn.sigmoid(x)
def _layernorm(x, axis=-1, eps=1e-5):
    m = jnp.mean(x, axis=axis, keepdims=True)
    v = jnp.var(x, axis=axis, keepdims=True)
    return (x - m) / jnp.sqrt(v + eps)
def _scatter_add(tgt, idx, src, axis=0):
    return tgt.at[idx].add(src)
def _segment_sum(src, seg, n):
    return jax.ops.segment_sum(src, seg, n)
class _Rng:
    def __init__(self, key):
        self._k = key
    def _next(self):
        self._k, sub = jax.random.split(self._k)
        return sub
    def normal(self, shape):
        return jax.random.normal(self._next(), shape, dtype=jnp.bfloat16)
    def randint(self, lo, hi, shape):
        return jax.random.randint(self._next(), shape, lo, hi, dtype=jnp.int32)
    def uniform(self, shape, lo=0.0, hi=1.0):
        return jax.random.uniform(self._next(), shape, jnp.bfloat16, lo, hi)
    def permutation(self, n):
        return jax.random.permutation(self._next(), n)


kernel_name = 'sequential_preLN__linear_kernel_hedgehog__dense_activation_squared_relu__prompt'

def setup_inputs():
    _rng = _Rng(jax.random.key(int.from_bytes(__import__("os").urandom(4), "little")))
    _w = (lambda a: (lambda t: t.astype(jnp.bfloat16) if jnp.issubdtype(t.dtype, jnp.floating) else t)(jnp.asarray(a)))
    def _A_setup():
        B, S, D, H = 1, 2048, 512, 32
        Dh = D // H
        return {
            "x": _w((lambda *s: _rng.normal(s) * 0.05)(B, S, D)),
            "wqkv": _w((lambda *s: _rng.normal(s) * 0.2)(D, 3 * D)),
            "w_phi": _w((lambda *s: _rng.normal(s) * 0.2)(H, Dh, Dh) * (Dh ** -0.5)),
            "wo": _w((lambda *s: _rng.normal(s) * 0.05)(D, D)),
        }
    _A_in = _A_setup()

    def _B_setup():
        B, S, D, F = 1, 2048, 512, 1792
        return {
            "x": _w((lambda *s: _rng.normal(s) * 0.05)(B, S, D)),
            "w1": _w((lambda *s: _rng.normal(s) * 0.05)(D, F)),
            "b1": _w((lambda *s: _rng.normal(s) * 0.05)(F)),
            "w2": _w((lambda *s: _rng.normal(s) * 0.05)(F, D)),
            "b2": _w((lambda *s: _rng.normal(s) * 0.05)(D)),
        }
    _B_in = _B_setup()

    return {
        "A_x": _A_in["x"],
        "A_wqkv": _A_in["wqkv"],
        "A_w_phi": _A_in["w_phi"],
        "A_wo": _A_in["wo"],
        "B_x": _B_in["x"],
        "B_w1": _B_in["w1"],
        "B_b1": _B_in["b1"],
        "B_w2": _B_in["w2"],
        "B_b2": _B_in["b2"],
    }

def reference(A_x, A_wqkv, A_w_phi, A_wo, B_x, B_w1, B_b1, B_w2, B_b2):
    def _A_ref(x, wqkv, w_phi, wo):
        B, S, D = x.shape
        H = 32; Dh = D // H
        qkv = (lambda x, *d: x.transpose(*d))((x @ wqkv).reshape(B, S, 3, H, Dh), 2, 0, 3, 1, 4)
        q, k, v = qkv[0], qkv[1], qkv[2]
        pq = jnp.einsum("bhsd,hdf->bhsf", q, w_phi)
        pk = jnp.einsum("bhsd,hdf->bhsf", k, w_phi)
        phi_q = jnp.concatenate([_softmax(pq, axis=-1), _softmax(-pq, axis=-1)], axis=-1)
        phi_k = jnp.concatenate([_softmax(pk, axis=-1), _softmax(-pk, axis=-1)], axis=-1)
        kv = jnp.einsum("bhsf,bhsd->bhfd", phi_k, v)
        z  = jnp.einsum("bhsf->bhf", phi_k)
        num = jnp.einsum("bhqf,bhfd->bhqd", phi_q, kv)
        den = jnp.einsum("bhqf,bhf->bhq", phi_q, z)[..., None] + 1e-6
        o = num / den
        return (lambda x, *d: x.transpose(*d))(o, 0, 2, 1, 3).reshape(B, S, D) @ wo

    def _B_ref(x, w1, b1, w2, b2):
        h = jnp.einsum("bsd,df->bsf", x, w1) + b1
        zero = jnp.zeros_like(h)
        r = jnp.where(h > zero, h, zero)
        h = r * r
        out = jnp.einsum("bsf,fd->bsd", h, w2) + b2
        return out

    x = A_x
    h = x + _A_ref(_layernorm(x, axis=-1), A_wqkv, A_w_phi, A_wo)
    h2 = h + _B_ref(_layernorm(h, axis=-1), B_w1, B_b1, B_w2, B_b2)
    return h2
```

```python
import functools
import math

import jax
import jax.numpy as jnp
from jax import lax
import jax.experimental.pallas as pl
import jax.experimental.pallas.tpu as pltpu

F32 = jnp.float32
BF16 = jnp.bfloat16
LOG2E = math.log2(math.e)
NT = (((1,), (1,)), ((), ()))
TN = (((0,), (0,)), ((), ()))


def _iota(shape, dim):
    return lax.broadcasted_iota(jnp.int32, shape, dim)


def _ln(x):
    m = jnp.mean(x, axis=-1, keepdims=True)
    xc = x - m
    v = jnp.mean(xc * xc, axis=-1, keepdims=True)
    return xc * lax.rsqrt(v + 1e-5)


def _softmax_pm(p, T):
    p3 = p.reshape(16, 8, T)
    mx = jnp.max(p3, axis=0, keepdims=True)
    mn = jnp.min(p3, axis=0, keepdims=True)
    ep = jnp.exp2(p3 - mx)
    en = jnp.exp2(mn - p3)
    rp = 1.0 / jnp.sum(ep, axis=0, keepdims=True)
    rn = 1.0 / jnp.sum(en, axis=0, keepdims=True)
    return (ep * rp).reshape(128, T), (en * rn).reshape(128, T)


def make_kernel(S, D, F, T):
    G = D // 128

    def kern(x_ref, wqkv_ref, wphi_ref, wo_ref, w1_ref, b1_ref, w2_ref, b2_ref, o_ref,
             wt_ref, wop_ref, phiq_ref, kv_ref, z_ref, l_ref):
        r = _iota((128, 128), 0)
        c = _iota((128, 128), 1)
        et = (_iota((128, 16), 0) // 8 == _iota((128, 16), 1)).astype(BF16)
        perm = ((r // 8 == c % 16) & (r % 8 == c // 16)).astype(BF16)
        hmask = (r % 8) == (c // 16)
        for g in range(G):
            sl = slice(g * 128, (g + 1) * 128)
            wg = wphi_ref[sl, :]
            rr = lax.dot_general(et, wg, NT, preferred_element_type=F32)
            bt = jnp.where(hmask, rr, 0.0).astype(BF16)
            for part in range(2):
                w = wqkv_ref[:, part * D + g * 128: part * D + (g + 1) * 128]
                wt_ref[part * D + g * 128: part * D + (g + 1) * 128, :] = (
                    lax.dot_general(bt, w, NT, preferred_element_type=F32) * LOG2E).astype(BF16)
            w = wqkv_ref[:, 2 * D + g * 128: 2 * D + (g + 1) * 128]
            wt_ref[2 * D + g * 128: 2 * D + (g + 1) * 128, :] = lax.dot_general(
                perm, w, NT, preferred_element_type=F32).astype(BF16)
            wop_ref[sl, :] = jnp.dot(perm, wo_ref[sl, :], preferred_element_type=F32).astype(BF16)

        kv_ref[...] = jnp.zeros_like(kv_ref)
        z_ref[...] = jnp.zeros_like(z_ref)

        for i in range(S // T):
            rows = slice(i * T, (i + 1) * T)
            xn = _ln(x_ref[rows, :].astype(F32)).astype(BF16)
            pt = lax.dot_general(wt_ref[...], xn, NT, preferred_element_type=F32)
            for g in range(G):
                qp, qn = _softmax_pm(pt[g * 128:(g + 1) * 128], T)
                phiq_ref[g * 256:g * 256 + 128, rows] = qp.astype(BF16)
                phiq_ref[g * 256 + 128:(g + 1) * 256, rows] = qn.astype(BF16)
                kp, kn = _softmax_pm(pt[D + g * 128:D + (g + 1) * 128], T)
                phk = jnp.concatenate([kp, kn], axis=0)
                vt = pt[2 * D + g * 128:2 * D + (g + 1) * 128].astype(BF16)
                kv_ref[g * 256:(g + 1) * 256, :] += lax.dot_general(
                    phk.astype(BF16), vt, NT, preferred_element_type=F32)
                zz = phk[:, 0:128]
                for j in range(1, T // 128):
                    zz = zz + phk[:, j * 128:(j + 1) * 128]
                z_ref[g * 256:(g + 1) * 256, :] += zz

        r2 = _iota((256, 128), 0)
        c2 = _iota((256, 128), 1)
        for g in range(G):
            kvg = jnp.where(r2 % 8 == c2 % 8, kv_ref[g * 256:(g + 1) * 256, :], 0.0)
            l_ref[g * 144:g * 144 + 128, :] = kvg.T.astype(BF16)
            zs = jnp.sum(z_ref[g * 256:(g + 1) * 256, :], axis=1, keepdims=True)
            zb = jnp.where(r2 % 8 == c2, jnp.broadcast_to(zs, (256, 128)), 0.0)
            l_ref[g * 144 + 128:(g + 1) * 144, :] = zb.T[0:16, :].astype(BF16)

        b1 = b1_ref[...].astype(F32)
        b2 = b2_ref[...].astype(F32)
        for i in range(S // T):
            rows = slice(i * T, (i + 1) * T)
            ots = []
            for g in range(G):
                res = jnp.dot(l_ref[g * 144:(g + 1) * 144, :], phiq_ref[g * 256:(g + 1) * 256, rows],
                              preferred_element_type=F32)
                rd = 1.0 / (res[128:136] + 1e-6)
                ots.append((res[:128].reshape(16, 8, T) * rd[None]).reshape(128, T).astype(BF16))
            ot = jnp.concatenate(ots, axis=0)
            attn = lax.dot_general(ot, wop_ref[...], TN, preferred_element_type=F32)
            h = x_ref[rows, :].astype(F32) + attn
            hn = _ln(h).astype(BF16)
            a = jnp.dot(hn, w1_ref[...], preferred_element_type=F32) + b1
            a = jnp.maximum(a, 0.0)
            a = (a * a).astype(BF16)
            out = jnp.dot(a, w2_ref[...], preferred_element_type=F32) + b2 + h
            o_ref[rows, :] = out.astype(o_ref.dtype)

    return kern


@jax.jit
def pallas_sequential_preLN__linear_kernel_hedgehog__dense_activation_squared_relu__prompt_kernel(
    A_x: jax.Array,
    A_wqkv: jax.Array,
    A_w_phi: jax.Array,
    A_wo: jax.Array,
    B_x: jax.Array,
    B_w1: jax.Array,
    B_b1: jax.Array,
    B_w2: jax.Array,
    B_b2: jax.Array,
):
    B, S, D = A_x.shape
    F = B_w1.shape[1]
    H, Dh, _ = A_w_phi.shape
    T = 512
    out = pl.pallas_call(
        make_kernel(S, D, F, T),
        out_shape=jax.ShapeDtypeStruct((S, D), A_x.dtype),
        scratch_shapes=[
            pltpu.VMEM((3 * D, D), BF16),
            pltpu.VMEM((D, D), BF16),
            pltpu.VMEM((2 * D, S), BF16),
            pltpu.VMEM((2 * D, 128), F32),
            pltpu.VMEM((2 * D, 128), F32),
            pltpu.VMEM((4 * 144, 256), BF16),
        ],
        compiler_params=pltpu.CompilerParams(vmem_limit_bytes=100 * 1024 * 1024),
    )(A_x.reshape(S, D), A_wqkv, A_w_phi.reshape(H * Dh, Dh), A_wo, B_w1,
      B_b1.reshape(1, F), B_w2, B_b2.reshape(1, D))
    return out.reshape(B, S, D)
```

```python
import functools
import math

import jax
import jax.numpy as jnp
from jax import lax
import jax.experimental.pallas as pl
import jax.experimental.pallas.tpu as pltpu

F32 = jnp.float32
BF16 = jnp.bfloat16
LOG2E = math.log2(math.e)
NT = (((1,), (1,)), ((), ()))
TN = (((0,), (0,)), ((), ()))


def _iota(shape, dim):
    return lax.broadcasted_iota(jnp.int32, shape, dim)


def _nt(a, b):
    return lax.dot_general(a, b, NT, preferred_element_type=F32)


def _dot(a, b):
    return jnp.dot(a, b, preferred_element_type=F32)


def _ln(x):
    m = jnp.mean(x, axis=-1, keepdims=True)
    xc = x - m
    v = jnp.mean(xc * xc, axis=-1, keepdims=True)
    return xc * lax.rsqrt(v + 1e-5)


def _softmax_pm(p):
    T = p.shape[1]
    p3 = p.reshape(8, 8, T)
    mx = jnp.max(p3, axis=0)
    mx = jnp.maximum(mx, pltpu.roll(mx, 4, 0))
    mn = jnp.min(p3, axis=0)
    mn = jnp.minimum(mn, pltpu.roll(mn, 4, 0))
    ep = jnp.exp2(p3 - mx[None])
    en = jnp.exp2(mn[None] - p3)
    sp = jnp.sum(ep, axis=0)
    sp = sp + pltpu.roll(sp, 4, 0)
    sn = jnp.sum(en, axis=0)
    sn = sn + pltpu.roll(sn, 4, 0)
    rp = 1.0 / sp
    rn = 1.0 / sn
    return (ep * rp[None]).reshape(64, T), (en * rn[None]).reshape(64, T)


def make_kernel(S, D, F, T1, T2):
    G4 = D // 64
    NB1 = S // T1
    NB2 = S // T2

    def kern(x_hbm, wqkv_hbm, wphi_hbm, wo_hbm, w1_hbm, b1_hbm, w2_hbm, b2_hbm, o_hbm,
             x_v, wqkv_v, wphi_v, wo_v, w1_v, b1_v, w2_v, b2_v, o_v,
             wt_ref, phiq_ref, kv_ref, z_ref, l_ref, sem):
        cx = [pltpu.make_async_copy(x_hbm.at[pl.ds(i * T1, T1), :], x_v.at[pl.ds(i * T1, T1), :], sem.at[i])
              for i in range(NB1)]
        n = NB1
        cw = [pltpu.make_async_copy(wqkv_hbm.at[:, pl.ds(p * D, D)], wqkv_v.at[p], sem.at[n + p])
              for p in range(3)]
        n += 3
        cphi = pltpu.make_async_copy(wphi_hbm, wphi_v, sem.at[n])
        cwo = pltpu.make_async_copy(wo_hbm, wo_v, sem.at[n + 1])
        cw1 = pltpu.make_async_copy(w1_hbm, w1_v, sem.at[n + 2])
        cb1 = pltpu.make_async_copy(b1_hbm, b1_v, sem.at[n + 3])
        cw2 = pltpu.make_async_copy(w2_hbm, w2_v, sem.at[n + 4])
        cb2 = pltpu.make_async_copy(b2_hbm, b2_v, sem.at[n + 5])
        n += 6
        co = [pltpu.make_async_copy(o_v.at[pl.ds(i * T2, T2), :], o_hbm.at[pl.ds(i * T2, T2), :], sem.at[n + i])
              for i in range(NB2)]

        cphi.start()
        cx[0].start()
        cw[2].start()
        cw[1].start()
        cw[0].start()
        for i in range(1, NB1):
            cx[i].start()
        cwo.start()
        cb1.start()
        cb2.start()
        cw1.start()
        cw2.start()

        cphi.wait()
        rep = (_iota((D, 32), 0) // 16 == _iota((D, 32), 1)).astype(BF16)
        y = _nt(rep, wphi_v[...])
        y = jnp.where(_iota((D, 256), 0) % 16 == _iota((D, 256), 1) // 16, y, 0.0).astype(BF16)
        lsel = ((_iota((128, 256), 0) % 64) // 4 == _iota((128, 256), 1) % 16).astype(BF16)
        bt = _nt(lsel, y)
        r = _iota((128, D), 0)
        c = _iota((128, D), 1)
        bt = jnp.where((c // 16) % 8 == 4 * (r // 64) + r % 4, bt, 0.0).astype(BF16)

        def fold(p):
            for g in range(D // 128):
                sl = slice(g * 128, (g + 1) * 128)
                wt_ref[p * D + g * 128:p * D + (g + 1) * 128, :] = (
                    _nt(bt[:, sl], wqkv_v[p, :, sl]) * LOG2E).astype(BF16)

        for i in range(NB1):
            rows = slice(i * T1, (i + 1) * T1)
            cx[i].wait()
            xn = _ln(x_v[rows, :].astype(F32)).astype(BF16)
            if i == 0:
                cw[2].wait()
                wt_ref[2 * D:3 * D, :] = wqkv_v[2].T
            vt = _nt(wt_ref[2 * D:3 * D, :], xn).astype(BF16)
            if i == 0:
                cw[1].wait()
                fold(1)
            pk = _nt(wt_ref[D:2 * D, :], xn)
            if i == 0:
                cw[0].wait()
                fold(0)
            pq = _nt(wt_ref[0:D, :], xn)
            for g in range(G4):
                kp, kn = _softmax_pm(pk[g * 64:(g + 1) * 64])
                phk = jnp.concatenate([kp, kn], axis=0)
                kvn = _nt(vt[g * 64:(g + 1) * 64], phk.astype(BF16))
                zz = phk[:, 0:128]
                for j in range(1, T1 // 128):
                    zz = zz + phk[:, j * 128:(j + 1) * 128]
                if i == 0:
                    kv_ref[g * 64:(g + 1) * 64, :] = kvn
                    z_ref[g * 128:(g + 1) * 128, :] = zz
                else:
                    kv_ref[g * 64:(g + 1) * 64, :] += kvn
                    z_ref[g * 128:(g + 1) * 128, :] += zz
                qp, qn = _softmax_pm(pq[g * 64:(g + 1) * 64])
                phiq_ref[g * 128:g * 128 + 64, rows] = qp.astype(BF16)
                phiq_ref[g * 128 + 64:(g + 1) * 128, rows] = qn.astype(BF16)

        kmask = _iota((64, 128), 0) // 16 == _iota((64, 128), 1) % 4
        zmask = _iota((16, 128), 0) == _iota((16, 128), 1) % 4
        for g in range(G4):
            l_ref[g * 80:g * 80 + 64, :] = jnp.where(kmask, kv_ref[g * 64:(g + 1) * 64, :], 0.0).astype(BF16)
            zs = jnp.sum(z_ref[g * 128:(g + 1) * 128, :].T, axis=0, keepdims=True)
            l_ref[g * 80 + 64:(g + 1) * 80, :] = jnp.where(
                zmask, jnp.broadcast_to(zs, (16, 128)), 0.0).astype(BF16)

        cwo.wait()
        cb1.wait()
        cb2.wait()
        cw1.wait()
        cw2.wait()
        b1 = b1_v[...].astype(F32)
        b1 = jnp.concatenate([b1[j:j + 1, :] for j in range(F // 128)], axis=1)
        b2 = b2_v[...].astype(F32)
        b2 = jnp.concatenate([b2[j:j + 1, :] for j in range(D // 128)], axis=1)
        for i in range(NB2):
            rows = slice(i * T2, (i + 1) * T2)
            ots = []
            for g in range(G4):
                res = _dot(l_ref[g * 80:(g + 1) * 80, :], phiq_ref[g * 128:(g + 1) * 128, rows])
                rd = 1.0 / (res[64:72] + 1e-6)
                rdb = jnp.concatenate([jnp.broadcast_to(rd[h:h + 1], (16, T2)) for h in range(4)], axis=0)
                ots.append((res[:64] * rdb).astype(BF16))
            ot = jnp.concatenate(ots, axis=0)
            attn = lax.dot_general(ot, wo_v[...], TN, preferred_element_type=F32)
            h = x_v[rows, :].astype(F32) + attn
            hn = _ln(h).astype(BF16)
            a = _dot(hn, w1_v[...]) + b1
            a = jnp.maximum(a, 0.0)
            a = (a * a).astype(BF16)
            out = _dot(a, w2_v[...]) + b2 + h
            o_v[rows, :] = out.astype(o_v.dtype)
            co[i].start()
        for i in range(NB2):
            co[i].wait()

    return kern, NB1 + 9 + NB2


def build(T1=512, T2=512, interpret=False):
    @jax.jit
    def fn(A_x, A_wqkv, A_w_phi, A_wo, B_x, B_w1, B_b1, B_w2, B_b2):
        B, S, D = A_x.shape
        F = B_w1.shape[1]
        H, Dh, _ = A_w_phi.shape
        kern, nsem = make_kernel(S, D, F, T1, T2)
        hbm = lambda a: pltpu.with_memory_space_constraint(a, pltpu.HBM) if not interpret else a
        out = pl.pallas_call(
            kern,
            out_shape=jax.ShapeDtypeStruct((S, D), A_x.dtype),
            in_specs=[pl.BlockSpec(memory_space=pltpu.HBM)] * 8,
            out_specs=pl.BlockSpec(memory_space=pltpu.HBM),
            scratch_shapes=[
                pltpu.VMEM((S, D), BF16),
                pltpu.VMEM((3, D, D), BF16),
                pltpu.VMEM((Dh * Dh, H), BF16),
                pltpu.VMEM((D, D), BF16),
                pltpu.VMEM((D, F), BF16),
                pltpu.VMEM((F // 128, 128), BF16),
                pltpu.VMEM((F, D), BF16),
                pltpu.VMEM((D // 128, 128), BF16),
                pltpu.VMEM((S, D), A_x.dtype),
                pltpu.VMEM((3 * D, D), BF16),
                pltpu.VMEM((2 * D, S), BF16),
                pltpu.VMEM((D, 128), F32),
                pltpu.VMEM((2 * D, 128), F32),
                pltpu.VMEM((8 * 80, 128), BF16),
                pltpu.SemaphoreType.DMA((nsem,)),
            ],
            compiler_params=pltpu.CompilerParams(vmem_limit_bytes=100 * 1024 * 1024),
            interpret=interpret,
        )(hbm(A_x.reshape(S, D)), hbm(A_wqkv), hbm(A_w_phi.transpose(1, 2, 0).reshape(Dh * Dh, H)), hbm(A_wo),
          hbm(B_w1), hbm(B_b1.reshape(F // 128, 128)), hbm(B_w2), hbm(B_b2.reshape(D // 128, 128)))
        return out.reshape(B, S, D)
    return fn


_impl = build(T1=512, T2=1024)


@jax.jit
def pallas_sequential_preLN__linear_kernel_hedgehog__dense_activation_squared_relu__prompt_kernel(
    A_x: jax.Array,
    A_wqkv: jax.Array,
    A_w_phi: jax.Array,
    A_wo: jax.Array,
    B_x: jax.Array,
    B_w1: jax.Array,
    B_b1: jax.Array,
    B_w2: jax.Array,
    B_b2: jax.Array,
):
    return _impl(A_x, A_wqkv, A_w_phi, A_wo, B_x, B_w1, B_b1, B_w2, B_b2)
```

```python
import math

import jax
import jax.numpy as jnp
from jax import lax
import jax.experimental.pallas as pl
import jax.experimental.pallas.tpu as pltpu

F32 = jnp.float32
BF16 = jnp.bfloat16
LOG2E = math.log2(math.e)
NT = (((1,), (1,)), ((), ()))
TN = (((0,), (0,)), ((), ()))


def _iota(shape, dim):
    return lax.broadcasted_iota(jnp.int32, shape, dim)


def _nt(a, b):
    return lax.dot_general(a, b, NT, preferred_element_type=F32)


def _dot(a, b):
    return jnp.dot(a, b, preferred_element_type=F32)


U32 = jnp.uint32


def _unp(x, e):
    return pltpu.unpack_elementwise(x, index=e, packed_dtype=BF16, unpacked_dtype=F32)


def _ln(x):
    m = jnp.mean(x, axis=-1, keepdims=True)
    xc = x - m
    v = jnp.mean(xc * xc, axis=-1, keepdims=True)
    return xc * lax.rsqrt(v + 1e-5)


def _softmax_pm(p):
    T = p.shape[1]
    p3 = p.reshape(8, 8, T)
    mx = jnp.max(p3, axis=0)
    mx = jnp.maximum(mx, pltpu.roll(mx, 4, 0))
    mn = jnp.min(p3, axis=0)
    mn = jnp.minimum(mn, pltpu.roll(mn, 4, 0))
    ep = jnp.exp2(p3 - mx[None])
    en = jnp.exp2(mn[None] - p3)
    sp = jnp.sum(ep, axis=0)
    sp = sp + pltpu.roll(sp, 4, 0)
    sn = jnp.sum(en, axis=0)
    sn = sn + pltpu.roll(sn, 4, 0)
    rp = 1.0 / sp
    rn = 1.0 / sn
    return (ep * rp[None]).reshape(64, T), (en * rn[None]).reshape(64, T)


def make_kernel(S, D, F, T1, T2, PR, LR, RC, ORDER, LOOP1, QFIRST, WAT, PS1, PS2, PA, PB, NK, EARLY, TF):
    G4 = D // 64
    NB1 = S // T1
    NB2 = S // T2
    TH = T2 // 2
    DH = D // 2
    FH = F // 2
    SX = 0
    SW = SX + NB1
    SO = SW + 9
    NSEM = SO + 4 * 8

    def kern(x_hbm, wqkv_hbm, wphi_hbm, wo_hbm, w1_hbm, b1_hbm, w2_hbm, b2_hbm, o_hbm,
             x_v, wqkv_v, wphi_v, wo_v, w1_v, b1_v, w2_v, b2_v, o_v,
             xa_ref, xb_ref, phiq_ref, kv_ref, z_ref, w1s_ref, w2s_ref, h_ref, la_ref, sem):
        def cx(i):
            r = pl.ds(i * T1, T1)
            return pltpu.make_async_copy(x_hbm.at[r, :], x_v.at[r, :], sem.at[SX + i])

        def co(i, t0, T, c):
            r = pl.ds(t0, T)
            return [pltpu.make_async_copy(o_v.at[r, pl.ds(c0, 128)], o_hbm.at[r, pl.ds(c0, 128)],
                                          sem.at[SO + 4 * i + 2 * c + k])
                    for k, c0 in enumerate((c * 128, DH + c * 128))]

        def co_wait(i, t0, T):
            for c in range(2):
                for d in co(i, t0, T, c):
                    d.wait()

        cw = [pltpu.make_async_copy(wqkv_hbm.at[:, pl.ds(p * D, D)], wqkv_v.at[p], sem.at[SW + p])
              for p in range(3)]
        cphi = pltpu.make_async_copy(wphi_hbm, wphi_v, sem.at[SW + 3])
        cwo = pltpu.make_async_copy(wo_hbm, wo_v, sem.at[SW + 4])
        cw1 = pltpu.make_async_copy(w1_hbm, w1_v, sem.at[SW + 5])
        cb1 = pltpu.make_async_copy(b1_hbm, b1_v, sem.at[SW + 6])
        cw2 = pltpu.make_async_copy(w2_hbm, w2_v, sem.at[SW + 7])
        cb2 = pltpu.make_async_copy(b2_hbm, b2_v, sem.at[SW + 8])

        cphi.start()
        cw[1].start()
        for i in range(NK):
            cx(i).start()
        cw[0].start()
        cw[2].start()
        for i in range(NK, NB1):
            cx(i).start()
        cwo.start()
        cb1.start()
        cb2.start()
        cw1.start()
        cw2.start()

        kv_ref[...] = jnp.zeros_like(kv_ref)
        z_ref[...] = jnp.zeros_like(z_ref)

        if 1:
            cphi.wait()
        rep = (_iota((D, 32), 0) // 16 == _iota((D, 32), 1)).astype(BF16)
        y = _nt(rep, wphi_v[...])
        y = jnp.where(_iota((D, 256), 0) % 16 == _iota((D, 256), 1) // 16, y, 0.0).astype(BF16)
        lsel = ((_iota((128, 256), 0) % 64) // 4 == _iota((128, 256), 1) % 16).astype(BF16)
        bt = _nt(lsel, y)
        r_ = _iota((128, D), 0)
        c_ = _iota((128, D), 1)
        bt = jnp.where((c_ // 16) % 8 == 4 * (r_ // 64) + r_ % 4, bt, 0.0).astype(BF16)

        def fold(p):
            return jnp.concatenate(
                [(_nt(bt[:, g * 128:(g + 1) * 128], wqkv_v[p, :, g * 128:(g + 1) * 128]) * LOG2E).astype(BF16)
                 for g in range(D // 128)], axis=0)

        def ln1(i, xn_ref):
            for r in range(0, T1, 32):
                rows = pl.ds(pl.multiple_of(i * T1 + r, 32), 32)
                xn_ref[r:r + 32, :] = _ln(x_v[rows, :].astype(F32)).astype(BF16)

        def proj(p, xn):
            return _nt(wt[p], xn)

        def presum(w_ref, ws_ref, kh, nh):
            for r in range(0, kh, PR):
                for c in range(0, nh, 128):
                    b11 = w_ref[r:r + PR, c:c + 128].astype(F32)
                    b12 = w_ref[r:r + PR, nh + c:nh + c + 128].astype(F32)
                    b21 = w_ref[kh + r:kh + r + PR, c:c + 128].astype(F32)
                    b22 = w_ref[kh + r:kh + r + PR, nh + c:nh + c + 128].astype(F32)
                    ws_ref[0, r:r + PR, c:c + 128] = (b11 + b22).astype(BF16)
                    ws_ref[1, r:r + PR, c:c + 128] = (b12 - b22).astype(BF16)
                    ws_ref[2, r:r + PR, c:c + 128] = (b21 - b11).astype(BF16)
                    ws_ref[3, r:r + PR, c:c + 128] = (b11 + b12).astype(BF16)
                    ws_ref[4, r:r + PR, c:c + 128] = (b21 + b22).astype(BF16)

        def tile(i, cur, nxt_ref, phk=None, ORDER=None):
            static = isinstance(i, int)
            nxt = min(i + 1, NB1 - 1) if static else jnp.minimum(i + 1, NB1 - 1)
            nt1 = T1 // 128
            xs = [cur[t * 128:(t + 1) * 128, :] for t in range(nt1)]
            if nxt_ref is not None and (not static or i + 1 < NB1):
                ln1(nxt, nxt_ref)

            def kpart():
                phk = [[] for _ in range(G4)]
                zz = [None] * G4
                for t in range(nt1):
                    pk = proj(1, xs[t])
                    for g in range(G4):
                        kp, kn = _softmax_pm(pk[g * 64:(g + 1) * 64])
                        ph = jnp.concatenate([kp, kn], axis=0)
                        zz[g] = ph if t == 0 else zz[g] + ph
                        phk[g].append(ph.astype(BF16))
                for g in range(G4):
                    z_ref[g * 128:(g + 1) * 128, :] += zz[g]
                return [jnp.concatenate(p, axis=1) for p in phk]

            def vpart():
                return jnp.concatenate([proj(2, xs[t]).astype(BF16) for t in range(nt1)], axis=1)

            def qpart():
                for t in range(nt1):
                    pq = proj(0, xs[t])
                    cols = pl.ds(pl.multiple_of(i * T1 + t * 128, 128), 128)
                    for g in range(G4):
                        qp, qn = _softmax_pm(pq[g * 64:(g + 1) * 64])
                        phiq_ref[g * 128:g * 128 + 64, cols] = qp.astype(BF16)
                        phiq_ref[g * 128 + 64:(g + 1) * 128, cols] = qn.astype(BF16)

            def kvpart(vt, phk):
                for g in range(G4):
                    kv_ref[g * 64:(g + 1) * 64, :] += _nt(vt[g * 64:(g + 1) * 64], phk[g])

            for ch in ("K" if ORDER else QFIRST):
                if ch == "K":
                    if phk is None:
                        phk = kpart()
                    if ORDER == "Konly":
                        return phk
                elif ch == "V":
                    vt = vpart()
                elif ch == "Q":
                    qpart()
                else:
                    kvpart(vt, phk)

        def phase1(j):
            if isinstance(j, int):
                cx(2 * j + 1).wait()
                if 2 * j + 2 < NB1:
                    cx(2 * j + 2).wait()
            else:
                cx(2 * j + 1).wait()

                @pl.when(2 * j + 2 < NB1)
                def _():
                    cx(jnp.minimum(2 * j + 2, NB1 - 1)).wait()
            tile(2 * j, xa_ref, xb_ref)
            tile(2 * j + 1, xb_ref, xa_ref)

        cw[1].wait()
        for i in range(NK):
            cx(i).wait()
        wt = [None] * 3
        wt[1] = fold(1)
        def lnv(i):
            return jnp.concatenate([_ln(x_v[i * T1 + r:i * T1 + r + 32, :].astype(F32)).astype(BF16)
                                    for r in range(0, T1, 32)], axis=0)
        xn0 = [lnv(i) for i in range(NK)]
        ph0 = [tile(i, xn0[i], None, ORDER="Konly") for i in range(NK)]
        cw[0].wait()
        cw[2].wait()
        cx(NK).wait()
        cx(NK + 1).wait()
        wt[0] = fold(0)
        wt[2] = wqkv_v[2].T
        def late_waits():
            cwo.wait()
            cb1.wait()
            cb2.wait()
            cw1.wait()
            cw2.wait()

        if LOOP1:
            pl.loop(0, NB1 // 2)(phase1)
            late_waits()
        else:
            for i in range(NB1):
                if i == NK + 1:
                    for j in range(NK + 2, NB1):
                        cx(j).wait()
                if i == WAT:
                    late_waits()
                if i == PS1:
                    presum(w1_v, w1s_ref, DH, FH)
                if i == PS2:
                    presum(w2_v, w2s_ref, FH, DH)
                if i < NK:
                    tile(i, xn0[i], xa_ref if i == NK - 1 else None, phk=ph0[i])
                else:
                    tile(i, *((xa_ref, xb_ref) if i % 2 == 0 else (xb_ref, xa_ref)))
            if WAT == NB1:
                late_waits()
        lmat = []
        kmask = _iota((64, 128), 0) // 16 == _iota((64, 128), 1) % 4
        zmask = _iota((16, 128), 0) == _iota((16, 128), 1) % 4
        for g in range(G4):
            kvm = jnp.where(kmask, kv_ref[g * 64:(g + 1) * 64, :], 0.0)
            zs = jnp.sum(z_ref[g * 128:(g + 1) * 128, :].T, axis=0, keepdims=True)
            zm = jnp.where(zmask, jnp.broadcast_to(zs, (16, 128)), 0.0)
            lmat.append(jnp.concatenate([kvm, zm], axis=0).astype(BF16))

        b1 = b1_v[...].astype(F32)
        b1 = jnp.concatenate([b1[j:j + 1, :] for j in range(F // 128)], axis=1)
        b2 = b2_v[...].astype(F32)
        b2 = jnp.concatenate([b2[j:j + 1, :] for j in range(D // 128)], axis=1)

        def numden(i):
            rows = slice(i * T2, (i + 1) * T2)
            ots = []
            for g in range(G4):
                res = _dot(lmat[g], phiq_ref[g * 128:(g + 1) * 128, rows])
                rd = 1.0 / (res[64:72] + 1e-6)
                rdb = jnp.concatenate([jnp.broadcast_to(rd[h:h + 1], (16, T2)) for h in range(4)], axis=0)
                ots.append((res[:64] * rdb).astype(BF16))
            return jnp.concatenate(ots, axis=0)

        def rhs(w_ref, ws_ref, kh, nh, cs):
            c0, c1 = cs
            return [ws_ref[0, :, c0:c1], w_ref[0:kh, c0:c1], ws_ref[1, :, c0:c1], ws_ref[2, :, c0:c1],
                    w_ref[kh:2 * kh, nh + c0:nh + c1], ws_ref[3, :, c0:c1], ws_ref[4, :, c0:c1]]

        def lhs(a11, a12, a21, a22):
            return [(a11 + a22).astype(BF16), (a21 + a22).astype(BF16), a11.astype(BF16), a22.astype(BF16),
                    (a11 + a12).astype(BF16), (a21 - a11).astype(BF16), (a12 - a22).astype(BF16)]

        def combine(m):
            m1, m2, m3, m4, m5, m6, m7 = m
            return m1 + m4 - m5 + m7, m3 + m5, m2 + m4, m1 - m2 + m3 + m6

        def relu2(a):
            a = jnp.maximum(a, 0.0)
            return a * a

        def mix(i, ot):
            for q in range(T2 // 128):
                r0 = i * T2 + q * 128
                attn = lax.dot_general(ot[:, q * 128:(q + 1) * 128], wo_v[...], TN,
                                       preferred_element_type=F32)
                for r in range(0, 64, LR):
                    ht = x_v[r0 + r:r0 + r + LR, :].astype(F32) + attn[r:r + LR]
                    hb = x_v[r0 + 64 + r:r0 + 64 + r + LR, :].astype(F32) + attn[64 + r:64 + r + LR]
                    h_ref[r0 + r:r0 + r + LR, :] = ht
                    h_ref[r0 + 64 + r:r0 + 64 + r + LR, :] = hb
                    nt, nb = _ln(ht), _ln(hb)
                    for j, v in enumerate(lhs(nt[:, :DH], nt[:, DH:], nb[:, :DH], nb[:, DH:])):
                        la_ref[j, r0 // 2 + r:r0 // 2 + r + LR, :] = v

        def ffn(i, t0, T):
            TH = T // 2
            if isinstance(t0, int):
                h0 = t0 // 2
            else:
                h0 = pl.multiple_of(t0 // 2, 64)
                t0 = pl.multiple_of(t0, 128)
            la = [la_ref[j, pl.ds(h0, TH), :] for j in range(7)]
            acts = [[] for _ in range(7)]
            for c in range(FH // 128):
                cs = (c * 128, (c + 1) * 128)
                rb = rhs(w1_v, w1s_ref, DH, FH, cs)
                m = [_dot(la[j], rb[j]) for j in range(7)]
                bl = b1[:, cs[0]:cs[1]]
                br = b1[:, FH + cs[0]:FH + cs[1]]
                parts = [[] for _ in range(7)]
                for r in range(0, TH, RC):
                    c11, c12, c21, c22 = combine([v[r:r + RC] for v in m])
                    for j, v in enumerate(lhs(relu2(c11 + bl), relu2(c12 + br), relu2(c21 + bl), relu2(c22 + br))):
                        parts[j].append(v)
                for j in range(7):
                    acts[j].append(jnp.concatenate(parts[j], axis=0))
            acts = [jnp.concatenate(v, axis=1) for v in acts]
            for c in range(DH // 128):
                cs = (c * 128, (c + 1) * 128)
                rb = rhs(w2_v, w2s_ref, FH, DH, cs)
                m = [_dot(acts[j], rb[j]) for j in range(7)]
                for r in range(0, TH, RC):
                    q, rr = r // 64, r % 64
                    cq = combine([v[r:r + RC] for v in m])
                    for (cv, dr, c0) in zip(cq, (0, 0, 64, 64), (cs[0], DH + cs[0], cs[0], DH + cs[0])):
                        rows = pl.ds(t0 + q * 128 + dr + rr, RC)
                        o_v[rows, c0:c0 + 128] = (
                            cv + b2[:, c0:c0 + 128] + h_ref[rows, c0:c0 + 128]).astype(o_v.dtype)
                if EARLY:
                    for d in co(i, t0, T, c):
                        d.start()
            if not EARLY:
                for c in range(2):
                    for d in co(i, t0, T, c):
                        d.start()

        ot = [numden(i) for i in range(NB2)]
        if PS1 == NB1:
            presum(w1_v, w1s_ref, DH, FH)
        if PS2 == NB1:
            presum(w2_v, w2s_ref, FH, DH)
        for i in range(NB2):
            mix(i, ot[i])
        nmid = (S - PA - PB) // TF
        if PA:
            ffn(0, 0, PA)
        pl.loop(0, nmid)(lambda j: ffn(1 + j, PA + j * TF, TF))
        if PB:
            ffn(1 + nmid, S - PB, PB)
        if PA:
            co_wait(0, 0, PA)
        for j in range(nmid):
            co_wait(1 + j, PA + j * TF, TF)
        if PB:
            co_wait(1 + nmid, S - PB, PB)

    return kern, NSEM


def build(T1=128, T2=512, PR=32, LR=16, RC=32, ORDER=0, LOOP1=0, WAT=16, PS1=16, PS2=16, PA=0, PB=0, NK=2, EARLY=1, TF=512, QFIRST='QKVA', interpret=False):
    @jax.jit
    def fn(A_x, A_wqkv, A_w_phi, A_wo, B_x, B_w1, B_b1, B_w2, B_b2):
        B, S, D = A_x.shape
        F = B_w1.shape[1]
        H, Dh, _ = A_w_phi.shape
        kern, nsem = make_kernel(S, D, F, T1, T2, PR, LR, RC, ORDER, LOOP1, QFIRST, WAT, PS1, PS2, PA, PB, NK, EARLY, TF)
        hbm = lambda a: pltpu.with_memory_space_constraint(a, pltpu.HBM) if not interpret else a
        out = pl.pallas_call(
            kern,
            out_shape=jax.ShapeDtypeStruct((S, D), A_x.dtype),
            in_specs=[pl.BlockSpec(memory_space=pltpu.HBM)] * 8,
            out_specs=pl.BlockSpec(memory_space=pltpu.HBM),
            scratch_shapes=[
                pltpu.VMEM((S, D), BF16),
                pltpu.VMEM((3, D, D), BF16),
                pltpu.VMEM((Dh * Dh, H), BF16),
                pltpu.VMEM((D, D), BF16),
                pltpu.VMEM((D, F), BF16),
                pltpu.VMEM((F // 128, 128), BF16),
                pltpu.VMEM((F, D), BF16),
                pltpu.VMEM((D // 128, 128), BF16),
                pltpu.VMEM((S, D), A_x.dtype),
                pltpu.VMEM((T1, D), BF16),
                pltpu.VMEM((T1, D), BF16),
                pltpu.VMEM((2 * D, S), BF16),
                pltpu.VMEM((D, 128), F32),
                pltpu.VMEM((2 * D, 128), F32),
                pltpu.VMEM((5, D // 2, F // 2), BF16),
                pltpu.VMEM((5, F // 2, D // 2), BF16),
                pltpu.VMEM((S, D), F32),
                pltpu.VMEM((7, S // 2, D // 2), BF16),
                pltpu.SemaphoreType.DMA((nsem,)),
            ],
            compiler_params=pltpu.CompilerParams(vmem_limit_bytes=100 * 1024 * 1024),
            interpret=interpret,
        )(hbm(A_x.reshape(S, D)), hbm(A_wqkv), hbm(A_w_phi.transpose(1, 2, 0).reshape(Dh * Dh, H)), hbm(A_wo),
          hbm(B_w1), hbm(B_b1.reshape(F // 128, 128)), hbm(B_w2), hbm(B_b2.reshape(D // 128, 128)))
        return out.reshape(B, S, D)
    return fn


_impl = build()


@jax.jit
def pallas_sequential_preLN__linear_kernel_hedgehog__dense_activation_squared_relu__prompt_kernel(
    A_x: jax.Array,
    A_wqkv: jax.Array,
    A_w_phi: jax.Array,
    A_wo: jax.Array,
    B_x: jax.Array,
    B_w1: jax.Array,
    B_b1: jax.Array,
    B_w2: jax.Array,
    B_b2: jax.Array,
):
    return _impl(A_x, A_wqkv, A_w_phi, A_wo, B_x, B_w1, B_b1, B_w2, B_b2)
```
